```python
import os as _os
_os.environ.setdefault("JAX_PLATFORMS", "cpu")
import jax
import jax.numpy as jnp

def _softmax(x, axis=-1):
    return jax.nn.softmax(x, axis=axis)
def _gelu(x):
    return jax.nn.gelu(x, approximate=True)
def _silu(x):
    return jax.nn.silu(x)
def _sigmoid(x):
    return jax.nn.sigmoid(x)
def _layernorm(x, axis=-1, eps=1e-5):
    m = jnp.mean(x, axis=axis, keepdims=True)
    v = jnp.var(x, axis=axis, keepdims=True)
    return (x - m) / jnp.sqrt(v + eps)
def _scatter_add(tgt, idx, src, axis=0):
    return tgt.at[idx].add(src)
def _segment_sum(src, seg, n):
    return jax.ops.segment_sum(src, seg, n)
class _Rng:
    def __init__(self, key):
        self._k = key
    def _next(self):
        self._k, sub = jax.random.split(self._k)
        return sub
    def normal(self, shape):
        return jax.random.normal(self._next(), shape, dtype=jnp.bfloat16)
    def randint(self, lo, hi, shape):
        return jax.random.randint(self._next(), shape, lo, hi, dtype=jnp.int32)
    def uniform(self, shape, lo=0.0, hi=1.0):
        return jax.random.uniform(self._next(), shape, jnp.bfloat16, lo, hi)
    def permutation(self, n):
        return jax.random.permutation(self._next(), n)


kernel_name = 'standalone__dense_activation_gelu__prompt'

def setup_inputs():
    _rng = _Rng(jax.random.key(int.from_bytes(__import__("os").urandom(4), "little")))
    _w = (lambda a: (lambda t: t.astype(jnp.bfloat16) if jnp.issubdtype(t.dtype, jnp.floating) else t)(jnp.asarray(a)))
    B, S, D, F = 1, 2048, 640, 1728
    return {
        "x": _w((lambda *s: _rng.normal(s) * 0.05)(B, S, D)),
        "w1": _w((lambda *s: _rng.normal(s) * 0.05)(D, F) * (D ** -0.5)),
        "b1": _w((lambda *s: _rng.normal(s) * 0.05)(F) * 0.01),
        "w2": _w((lambda *s: _rng.normal(s) * 0.05)(F, D) * (F ** -0.5)),
        "b2": _w((lambda *s: _rng.normal(s) * 0.05)(D) * 0.01),
    }

def reference(x, w1, b1, w2, b2):
    h = jnp.einsum("bsd,df->bsf", x, w1) + b1
    h = _gelu(h)
    return jnp.einsum("bsf,fd->bsd", h, w2) + b2
```

```python
import functools
import math

import jax
import jax.numpy as jnp
from jax import lax
import jax.experimental.pallas as pl
import jax.experimental.pallas.tpu as pltpu

_LANE = 128
_NT = (((1,), (1,)), ((), ()))


def _gelu_tanh(h):
    c = math.sqrt(2.0 / math.pi)
    return 0.5 * h * (1.0 + jnp.tanh(c * (h + 0.044715 * (h * h * h))))


def _hidden(xt, w1_buf, f0, f1):
    f32 = jnp.float32
    fm = f0 + ((f1 - f0) // _LANE) * _LANE
    if fm == f1 or fm == f0:
        return lax.dot_general(xt, w1_buf[pl.ds(f0, f1 - f0), :], _NT,
                               preferred_element_type=f32)
    h_rest_t = lax.dot_general(w1_buf[pl.ds(fm, f1 - fm), :], xt, _NT,
                               preferred_element_type=f32)
    h_main = lax.dot_general(xt, w1_buf[pl.ds(f0, fm - f0), :], _NT,
                             preferred_element_type=f32)
    return jnp.concatenate([h_main, h_rest_t.T], axis=1)


def _kernel(x_hbm, w1t_hbm, b1_hbm, w2_hbm, b2_hbm, o_hbm,
            x_buf, w1_buf, w2_buf, b1_buf, b2_buf, b1f, b2f, o_buf,
            in_sem, out_sem, *, tm0, n_iter, sub, chunks):
    m_rows, _ = x_buf.shape
    f_dim = w1_buf.shape[0]
    nc = len(chunks)
    f32 = jnp.float32
    blk = sum(sub)
    assert tm0 + n_iter * blk == m_rows

    s_x0, s_xb, s_w1 = 0, 1, 3
    s_w2 = s_w1 + nc
    s_b = s_w2 + nc

    x0_copy = pltpu.make_async_copy(
        x_hbm.at[pl.ds(0, tm0), :], x_buf.at[pl.ds(0, tm0), :], in_sem.at[s_x0])

    def xb_copy(i):
        r = tm0 + i * blk
        return pltpu.make_async_copy(
            x_hbm.at[pl.ds(r, blk), :], x_buf.at[pl.ds(r, blk), :],
            in_sem.at[s_xb + i % 2])

    def w_copy(src, dst, j, base):
        f0, f1 = chunks[j]
        return pltpu.make_async_copy(
            src.at[pl.ds(f0, f1 - f0), :], dst.at[pl.ds(f0, f1 - f0), :],
            in_sem.at[base + j])

    w1_copy = lambda j: w_copy(w1t_hbm, w1_buf, j, s_w1)
    w2_copy = lambda j: w_copy(w2_hbm, w2_buf, j, s_w2)
    b1_copy = pltpu.make_async_copy(b1_hbm, b1_buf, in_sem.at[s_b])
    b2_copy = pltpu.make_async_copy(b2_hbm, b2_buf, in_sem.at[s_b + 1])

    def o_copy(r0, n, k):
        return pltpu.make_async_copy(
            o_buf.at[pl.ds(r0, n), :], o_hbm.at[pl.ds(r0, n), :], out_sem.at[k])

    def full_tile(r0, n):
        xt = x_buf[pl.ds(r0, n), :]
        h = _hidden(xt, w1_buf, 0, f_dim) + b1f[...]
        g = _gelu_tanh(h).astype(w2_buf.dtype)
        y = jnp.dot(g, w2_buf[...], preferred_element_type=f32)
        o_buf[pl.ds(r0, n), :] = (y + b2f[...]).astype(o_buf.dtype)

    b1_copy.start()
    b2_copy.start()
    x0_copy.start()
    w1_copy(0).start()
    w2_copy(0).start()
    for j in range(1, nc):
        w1_copy(j).start()
        w2_copy(j).start()
    xb_copy(0).start()

    x0_copy.wait()
    xt0 = x_buf[pl.ds(0, tm0), :]
    acc = None
    for j, (f0, f1) in enumerate(chunks):
        w1_copy(j).wait()
        h = _hidden(xt0, w1_buf, f0, f1)
        if j == 0:
            b1_copy.wait()
            b2_copy.wait()
            b1f[...] = b1_buf[...].astype(f32)[None, :]
            b2f[...] = b2_buf[...].astype(f32)[None, :]
        h = h + b1f[:, pl.ds(f0, f1 - f0)]
        g = _gelu_tanh(h).astype(w2_buf.dtype)
        w2_copy(j).wait()
        yj = jnp.dot(g, w2_buf[pl.ds(f0, f1 - f0), :], preferred_element_type=f32)
        acc = yj if acc is None else acc + yj
    o_buf[pl.ds(0, tm0), :] = (acc + b2f[...]).astype(o_buf.dtype)
    o_copy(0, tm0, 0).start()

    def body(i, carry):
        @pl.when(i + 1 < n_iter)
        def _():
            xb_copy(i + 1).start()

        xb_copy(i).wait()
        base = pl.multiple_of(tm0 + i * blk, _LANE)
        off = 0
        for n in sub:
            full_tile(base + off, n)
            o_copy(base + off, n, 1 + i).start()
            off += n
        return carry

    lax.fori_loop(0, n_iter, body, 0)

    o_copy(0, tm0, 0).wait()
    for i in range(n_iter):
        off = 0
        for n in sub:
            o_copy(tm0 + i * blk + off, n, 1 + i).wait()
            off += n


def _plan(m_rows, f_dim):
    tm0 = 256
    rest = m_rows - tm0
    n_iter = 2
    assert rest % (n_iter * _LANE) == 0, (m_rows,)
    blk = rest // n_iter
    sub = [256] * (blk // 256)
    if blk % 256:
        sub.append(blk % 256)
    sizes, f = [], 0
    for c in (128, 384, 512):
        if f + c < f_dim:
            sizes.append(c)
            f += c
    sizes.append(f_dim - f)
    bounds, f = [], 0
    for c in sizes:
        bounds.append((f, f + c))
        f += c
    return tm0, n_iter, tuple(sub), tuple(bounds)


@jax.jit
def pallas_standalone__dense_activation_gelu__prompt_kernel(
    x: jax.Array,
    w1: jax.Array,
    b1: jax.Array,
    w2: jax.Array,
    b2: jax.Array,
):
    B, S, D = x.shape
    F = w1.shape[1]
    M = B * S
    tm0, n_iter, sub, chunks = _plan(M, F)

    kernel = functools.partial(
        _kernel, tm0=tm0, n_iter=n_iter, sub=sub, chunks=chunks)
    hbm = pl.BlockSpec(memory_space=pl.ANY)
    out = pl.pallas_call(
        kernel,
        in_specs=[hbm] * 5,
        out_specs=hbm,
        out_shape=jax.ShapeDtypeStruct((M, D), x.dtype),
        scratch_shapes=[
            pltpu.VMEM((M, D), x.dtype),
            pltpu.VMEM((F, D), w1.dtype),
            pltpu.VMEM((F, D), w2.dtype),
            pltpu.VMEM((F,), b1.dtype),
            pltpu.VMEM((D,), b2.dtype),
            pltpu.VMEM((1, F), jnp.float32),
            pltpu.VMEM((1, D), jnp.float32),
            pltpu.VMEM((M, D), x.dtype),
            pltpu.SemaphoreType.DMA((3 + 2 * len(chunks) + 2,)),
            pltpu.SemaphoreType.DMA((1 + n_iter,)),
        ],
        compiler_params=pltpu.CompilerParams(vmem_limit_bytes=100 * 1024 * 1024),
    )(x.reshape(M, D), w1.T, b1, w2, b2)
    return out.reshape(B, S, D)
```
